```python
import jax
import jax.numpy as jnp

def _softmax(x, axis=-1):
    return jax.nn.softmax(x, axis=axis)

def _gelu(x):
    return jax.nn.gelu(x, approximate=True)

def _silu(x):
    return jax.nn.silu(x)

def _sigmoid(x):
    return jax.nn.sigmoid(x)

def _layernorm(x, axis=-1, eps=1e-05):
    m = jnp.mean(x, axis=axis, keepdims=True)
    v = jnp.var(x, axis=axis, keepdims=True)
    return (x - m) / jnp.sqrt(v + eps)

def _scatter_add(tgt, idx, src, axis=0):
    return tgt.at[idx].add(src)

def _segment_sum(src, seg, n):
    return jax.ops.segment_sum(src, seg, n)

class _Rng:

    def __init__(self, key):
        self._k = key

    def _next(self):
        self._k, sub = jax.random.split(self._k)
        return sub

    def normal(self, shape):
        return jax.random.normal(self._next(), shape, dtype=jnp.bfloat16)

    def randint(self, lo, hi, shape):
        return jax.random.randint(self._next(), shape, lo, hi, dtype=jnp.int32)

    def uniform(self, shape, lo=0.0, hi=1.0):
        return jax.random.uniform(self._next(), shape, jnp.bfloat16, lo, hi)

    def permutation(self, n):
        return jax.random.permutation(self._next(), n)
kernel_name = 'adaLN_cond__sliding_block_cached__geglu_ffn__decode'

def setup_inputs():
    _rng = _Rng(jax.random.key(int.from_bytes(__import__("os").urandom(4), "little")))
    _w = lambda a: (lambda t: t.astype(jnp.bfloat16) if jnp.issubdtype(t.dtype, jnp.floating) else t)(jnp.asarray(a))

    def _A_setup():
        B, Sq, D = (1, 1, 640)
        Hq, Hkv, Sk, Dh = (32, 32, 32768, 192)
        assert Hq % Hkv == 0, (Hq, Hkv)
        return {'x': _w((lambda *s: _rng.normal(s) * 0.05)(B, Sq, D)), 'k_cache': _w((lambda *s: _rng.normal(s) * 0.05)(B, Hkv, Sk, Dh)), 'v_cache': _w((lambda *s: _rng.normal(s) * 0.05)(B, Hkv, Sk, Dh)), 'wq': _w((lambda *s: _rng.normal(s) * 0.05)(D, Hq * Dh) * D ** (-0.5)), 'wo': _w((lambda *s: _rng.normal(s) * 0.05)(Hq * Dh, D) * (Hq * Dh) ** (-0.5))}
    _A_in = _A_setup()

    def _B_setup():
        B, S, D, F = (1, 1, 640, 1536)
        return {'x': _w((lambda *s: _rng.normal(s) * 0.05)(B, S, D)), 'w_gate': _w((lambda *s: _rng.normal(s) * 0.05)(D, F)), 'w_up': _w((lambda *s: _rng.normal(s) * 0.05)(D, F)), 'w_down': _w((lambda *s: _rng.normal(s) * 0.05)(F, D))}
    _B_in = _B_setup()
    return {'A_x': _A_in['x'], 'A_k_cache': _A_in['k_cache'], 'A_v_cache': _A_in['v_cache'], 'A_wq': _A_in['wq'], 'A_wo': _A_in['wo'], 'B_x': _B_in['x'], 'B_w_gate': _B_in['w_gate'], 'B_w_up': _B_in['w_up'], 'B_w_down': _B_in['w_down'], 'c': _w((lambda *s: _rng.normal(s) * 0.05)(1, 640)), 'w_mod': _w((lambda *s: _rng.normal(s) * 0.05)(640, 6 * 640) * 640 ** (-0.5))}

def reference(A_x, A_k_cache, A_v_cache, A_wq, A_wo, B_x, B_w_gate, B_w_up, B_w_down, c, w_mod):

    def _A_ref(x, k_cache, v_cache, wq, wo):
        B, Sq, D = x.shape
        Hq, Dh = (32, 192)
        Hkv, Sk = (k_cache.shape[1], k_cache.shape[2])
        W = min(4096, max(256, Sk // 4))
        rep = Hq // Hkv
        q = (lambda x, *d: x.transpose(*d))((x @ wq).reshape(B, Sq, Hq, Dh), 0, 2, 1, 3)
        k = jnp.repeat(k_cache[:, :, Sk - W:, :], rep, axis=1)
        v = jnp.repeat(v_cache[:, :, Sk - W:, :], rep, axis=1)
        scores = jnp.einsum('bhqd,bhkd->bhqk', q, k) * Dh ** (-0.5)
        p = _softmax(scores, axis=-1)
        o = jnp.einsum('bhqk,bhkd->bhqd', p, v)
        return (lambda x, *d: x.transpose(*d))(o, 0, 2, 1, 3).reshape(B, Sq, Hq * Dh) @ wo

    def _B_ref(x, w_gate, w_up, w_down):
        return _gelu(x @ w_gate) * (x @ w_up) @ w_down
    x = A_x
    mod = (_silu(c) @ w_mod).reshape(c.shape[0], 6, 1, -1)
    sa, ca, ga, sb, cb, gb = (mod[:, 0].copy(), mod[:, 1].copy(), mod[:, 2].copy(), mod[:, 3].copy(), mod[:, 4].copy(), mod[:, 5].copy())
    h = _layernorm(x, axis=-1) * (1 + ca) + sa
    x = x + ga * _A_ref(h, A_k_cache, A_v_cache, A_wq, A_wo)
    h = _layernorm(x, axis=-1) * (1 + cb) + sb
    x = x + gb * _B_ref(h, B_w_gate, B_w_up, B_w_down)
    return x
```

```python
import functools

import jax
import jax.numpy as jnp
import numpy as np
from jax import lax
from jax.experimental import pallas as pl
from jax.experimental.pallas import tpu as pltpu

F32 = jnp.float32
BF16 = jnp.bfloat16

D = 640
H = 32
DH = 192
F = 1536
WINDOW_MAX = 4096

ROWS = 8
SCH = 2048
LOOKAHEAD = 24
NSLOT = 48
PRIO = (0, 1, 1)


def _layernorm(x):
    m = jnp.mean(x, axis=-1, keepdims=True)
    xc = x - m
    v = jnp.mean(xc * xc, axis=-1, keepdims=True)
    return xc / jnp.sqrt(v + 1e-5)


def _bcast_rows(x):
    return jnp.broadcast_to(x, (8, x.shape[-1]))


def _kernel(x_hbm, c_hbm, k_hbm, v_hbm, wq_hbm, wo_hbm, wg_hbm, wu_hbm, wd_hbm, wm_hbm,
            o_ref,
            x_v, c_v, wm_v, wq_v, wo_v, wg_v, wu_v, wd_v, kv, qb, p_s, oacc, mod_s,
            sems, small_sems, *, sk, window):
    nr = DH // ROWS
    ns = window // SCH
    per_head = 2 * nr * ns
    assert per_head % NSLOT == 0 and per_head % len(PRIO) == 0 and LOOKAHEAD <= NSLOT
    w0 = sk - window

    def rows_of(hbm, vmem, step, c0=0, cw=None):
        n = hbm.shape[0]
        cw = hbm.shape[1] - c0 if cw is None else cw
        return [(hbm.at[pl.ds(r, step), pl.ds(c0, cw)], vmem.at[pl.ds(r, step), pl.ds(c0, cw)])
                for r in range(0, n, step)]

    def interleave(*lists):
        return [j for group in zip(*lists) for j in group]

    wm_jobs = interleave(rows_of(wm_hbm, wm_v, 8, 0, 3 * D), rows_of(wm_hbm, wm_v, 8, 3 * D, 3 * D))
    wq_jobs = interleave(*[rows_of(wq_hbm, wq_v, 8, c0, 2048) for c0 in (0, 2048, 4096)])
    wo_jobs = rows_of(wo_hbm, wo_v, 24)
    wg_jobs = rows_of(wg_hbm, wg_v, 8)
    wu_jobs = rows_of(wu_hbm, wu_v, 8)
    wd_jobs = rows_of(wd_hbm, wd_v, 16)
    pre = wm_jobs + wq_jobs + wo_jobs
    post = wg_jobs + wu_jobs + wd_jobs
    n_pre, n_post = len(pre), len(post)

    def prio(i):
        return PRIO[i % len(PRIO)]

    def pre_copy(i):
        src, dst = pre[i]
        return pltpu.make_async_copy(src, dst, sems.at[(i - n_pre) % NSLOT])

    def post_copy(i):
        src, dst = post[i]
        return pltpu.make_async_copy(src, dst, sems.at[i % NSLOT])

    def kv_copy(h, u):
        src = k_hbm if u < per_head // 2 else v_hbm
        s, r = divmod(u % (per_head // 2), nr)
        return pltpu.make_async_copy(
            src.at[h, pl.ds(r * ROWS, ROWS), pl.ds(w0 + s * SCH, SCH)],
            kv.at[u % NSLOT], sems.at[u % NSLOT])

    def pre_step(i):
        pre_copy(i).wait()
        j = i + LOOKAHEAD
        if j < n_pre:
            pre_copy(j).start(priority=prio(j - n_pre))
        else:
            kv_copy(0, j - n_pre).start(priority=prio(j - n_pre))

    def post_step(i):
        post_copy(i).wait()
        j = i + LOOKAHEAD
        if j < n_post:
            post_copy(j).start(priority=prio(j))

    x_cp = pltpu.make_async_copy(x_hbm, x_v, small_sems.at[0])
    c_cp = pltpu.make_async_copy(c_hbm, c_v, small_sems.at[1])
    c_cp.start()
    x_cp.start()
    for i in range(LOOKAHEAD):
        pre_copy(i).start(priority=prio(i - n_pre))
    c_cp.wait()
    x_cp.wait()
    c = _bcast_rows(c_v[...].astype(F32))
    sc = (c * jax.nn.sigmoid(c)).astype(BF16)
    x = _bcast_rows(x_v[...].astype(F32))
    lnx = _layernorm(x)

    step = 0
    n_blk = len(wm_jobs) // (D // 128)
    mod = jnp.zeros((8, 6 * D), F32)
    for kb in range(D // 128):
        for _ in range(n_blk):
            pre_step(step)
            step += 1
        mod = mod + jnp.dot(sc[:, kb * 128:(kb + 1) * 128], wm_v[kb * 128:(kb + 1) * 128, :],
                            preferred_element_type=F32)
    mod_s[...] = mod
    sa, ca = mod[:, 0:D], mod[:, D:2 * D]
    hq = (lnx * (1.0 + ca) + sa).astype(BF16)

    n_blk = len(wq_jobs) // (D // 128)
    q = jnp.zeros((8, H * DH), F32)
    for kb in range(D // 128):
        for _ in range(n_blk):
            pre_step(step)
            step += 1
        q = q + jnp.dot(hq[:, kb * 128:(kb + 1) * 128], wq_v[kb * 128:(kb + 1) * 128, :],
                        preferred_element_type=F32)
    q = q.astype(BF16).astype(F32) * np.float32(DH ** -0.5)

    n_qblk = H * DH // 128
    per_blk = len(wo_jobs) // n_qblk
    for b in range(n_qblk):
        for _ in range(per_blk):
            pre_step(step)
            step += 1
        qb[b * 128:(b + 1) * 128, :] = jnp.broadcast_to(q[0:1, b * 128:(b + 1) * 128], (128, 128)).T
    while step < n_pre:
        pre_step(step)
        step += 1

    def head(h, out_acc, last):
        def kv_step(u):
            kv_copy(h, u).wait()
            j = u + LOOKAHEAD
            if j < per_head:
                kv_copy(h, j).start(priority=prio(j))
            elif not last:
                kv_copy(h + 1, j - per_head).start(priority=prio(j))
            else:
                post_copy(j - per_head).start(priority=prio(j))
            return kv[u % NSLOT].astype(F32)

        row0 = h * DH
        u = 0
        for s in range(ns):
            acc = jnp.zeros((ROWS, SCH), F32)
            for r in range(nr):
                kt = kv_step(u)
                u += 1
                qv = qb[pl.ds(pl.multiple_of(row0 + r * ROWS, ROWS), ROWS), :]
                acc = acc + kt * jnp.tile(qv, (1, SCH // 128))
            p_s[:, s * SCH:(s + 1) * SCH] = _bcast_rows(jnp.sum(acc, axis=0, keepdims=True))
        sc_all = p_s[...]
        m = jnp.max(sc_all, axis=-1, keepdims=True)
        p = jnp.exp(sc_all - m)
        l = jnp.sum(p, axis=-1, keepdims=True)
        p_s[...] = p
        for s in range(ns):
            ps = p_s[:, s * SCH:(s + 1) * SCH]
            for r in range(nr):
                prod = kv_step(u) * ps
                u += 1
                parts = [prod[:, t * 128:(t + 1) * 128] for t in range(SCH // 128)]
                while len(parts) > 1:
                    parts = [parts[i] + parts[i + 1] for i in range(0, len(parts), 2)]
                if s == 0:
                    oacc[r * ROWS:(r + 1) * ROWS, :] = parts[0]
                else:
                    oacc[r * ROWS:(r + 1) * ROWS, :] += parts[0]
        o = jnp.sum(oacc[...], axis=-1, keepdims=True) / l[0:1, :]
        ob = jnp.broadcast_to(o, (DH, 128))
        for r in range(nr):
            wt = wo_v[pl.ds(pl.multiple_of(row0 + r * ROWS, ROWS), ROWS), :].astype(F32)
            out_acc = out_acc + wt * jnp.tile(ob[r * ROWS:(r + 1) * ROWS, :], (1, D // 128))
        return out_acc

    out_acc = lax.fori_loop(0, H - 1, lambda h, a: head(h, a, False), jnp.zeros((8, D), F32))
    out_acc = head(H - 1, out_acc, True)

    attn = _bcast_rows(jnp.sum(out_acc, axis=0, keepdims=True))
    ga, sb, cb, gb = (mod_s[:, i * D:(i + 1) * D] for i in (2, 3, 4, 5))
    x1 = x + ga * attn
    h2 = (_layernorm(x1) * (1.0 + cb) + sb).astype(BF16)

    step = 0
    for _ in range(len(wg_jobs)):
        post_step(step)
        step += 1
    g = jnp.dot(h2, wg_v[...], preferred_element_type=F32)
    for _ in range(len(wu_jobs)):
        post_step(step)
        step += 1
    up = jnp.dot(h2, wu_v[...], preferred_element_type=F32)
    act = (jax.nn.gelu(g, approximate=True) * up).astype(BF16)

    n_blk = len(wd_jobs) // (F // 128)
    y = jnp.zeros((8, D), F32)
    for kb in range(F // 128):
        for _ in range(n_blk):
            post_step(step)
            step += 1
        y = y + jnp.dot(act[:, kb * 128:(kb + 1) * 128], wd_v[kb * 128:(kb + 1) * 128, :],
                        preferred_element_type=F32)
    assert step == n_post
    o_ref[...] = (x1 + gb * y)[0:1, :].astype(o_ref.dtype)


@jax.jit
def pallas_adaLN_cond__sliding_block_cached__geglu_ffn__decode_kernel(
    A_x: jax.Array,
    A_k_cache: jax.Array,
    A_v_cache: jax.Array,
    A_wq: jax.Array,
    A_wo: jax.Array,
    B_x: jax.Array,
    B_w_gate: jax.Array,
    B_w_up: jax.Array,
    B_w_down: jax.Array,
    c: jax.Array,
    w_mod: jax.Array,
):
    del B_x
    _, hkv, sk, dh = A_k_cache.shape
    assert A_x.shape == (1, 1, D) and (hkv, dh) == (H, DH)
    window = min(WINDOW_MAX, max(256, sk // 4))
    assert window % SCH == 0

    k_t = jnp.transpose(A_k_cache, (0, 1, 3, 2)).reshape(H, DH, sk)
    v_t = jnp.transpose(A_v_cache, (0, 1, 3, 2)).reshape(H, DH, sk)

    hbm = pl.BlockSpec(memory_space=pl.ANY)
    out = pl.pallas_call(
        functools.partial(_kernel, sk=sk, window=window),
        out_shape=jax.ShapeDtypeStruct((1, D), A_x.dtype),
        in_specs=[hbm] * 10,
        out_specs=pl.BlockSpec(memory_space=pltpu.VMEM),
        scratch_shapes=[
            pltpu.VMEM((1, D), BF16),
            pltpu.VMEM((1, D), BF16),
            pltpu.VMEM((D, 6 * D), BF16),
            pltpu.VMEM((D, H * DH), BF16),
            pltpu.VMEM((H * DH, D), BF16),
            pltpu.VMEM((D, F), BF16),
            pltpu.VMEM((D, F), BF16),
            pltpu.VMEM((F, D), BF16),
            pltpu.VMEM((NSLOT, ROWS, SCH), BF16),
            pltpu.VMEM((H * DH, 128), F32),
            pltpu.VMEM((8, window), F32),
            pltpu.VMEM((DH, 128), F32),
            pltpu.VMEM((8, 6 * D), F32),
            pltpu.SemaphoreType.DMA((NSLOT,)),
            pltpu.SemaphoreType.DMA((2,)),
        ],
        compiler_params=pltpu.CompilerParams(vmem_limit_bytes=64 * 1024 * 1024),
        name="adaln_attn_geglu_decode",
    )(A_x.reshape(1, D), c, k_t, v_t, A_wq, A_wo, B_w_gate, B_w_up, B_w_down, w_mod)
    return out.reshape(1, 1, D)
```

```python
import functools

import jax
import jax.numpy as jnp
import numpy as np
from jax import lax
from jax.experimental import pallas as pl
from jax.experimental.pallas import tpu as pltpu

F32 = jnp.float32
BF16 = jnp.bfloat16

D = 640
H = 32
DH = 192
F = 1536
WINDOW_MAX = 4096

ROWS = 16
SCH = 512
LOOKAHEAD = 64
NSLOT = 96
PRIO = (0, 1, 1)
WM_JOB = (8, 1280, 24)
WQ_JOB = (8, 2048, 16)
WO_JOB = (24, 640, 16)
WGU_JOB = (8, 1536, 10)
WD_JOB = (16, 640, 1)
MOD_COLS = 768
Q_COLS = 512
FFN_COLS = 512
WD_SPLITS = (512, 1024, 1408, 1536)


def _layernorm(x):
    m = jnp.mean(x, axis=-1, keepdims=True)
    xc = x - m
    v = jnp.mean(xc * xc, axis=-1, keepdims=True)
    return xc / jnp.sqrt(v + 1e-5)


def _bcast_rows(x):
    return jnp.broadcast_to(x, (8, x.shape[-1]))


class _Stream:
    def __init__(self, jobs, first, budget, started=0):
        self.jobs, self.first, self.budget = jobs, first, budget
        self.waited, self.started = 0, started

    def fill(self):
        inflight = sum(n for _, n in self.jobs[self.waited:self.started])
        while self.started < len(self.jobs):
            make, n = self.jobs[self.started]
            if inflight + n > self.budget:
                break
            make().start(priority=PRIO[(self.first + self.started) % len(PRIO)])
            inflight += n
            self.started += 1

    def step(self, n=1):
        for _ in range(n):
            self.jobs[self.waited][0]().wait()
            self.waited += 1
            self.fill()


def _kernel(x_hbm, c_hbm, k_hbm, v_hbm, wq_hbm, wo_hbm, wg_hbm, wu_hbm, wd_hbm, wm_hbm,
            o_ref,
            x_v, c_v, wm_v, wq_v, wo_v, wg_v, wu_v, wd_v, kv, qb, p_s, mod_s,
            sems, small_sems, *, sk, window):
    nr = DH // ROWS
    ns = window // SCH
    per_head = 2 * nr * ns
    assert per_head % NSLOT == 0 and per_head % len(PRIO) == 0 and LOOKAHEAD <= NSLOT
    w0 = sk - window
    kv_bytes = ROWS * SCH * 2
    budget = LOOKAHEAD * kv_bytes

    def tiles(hbm, vmem, job):
        (rows, cols, stride), (n, m) = job, hbm.shape
        base = [(pl.ds(r, rows), pl.ds(c0, cols)) for r in range(0, n, rows) for c0 in range(0, m, cols)]
        return [(hbm.at[base[j]], vmem.at[base[j]])
                for k in range(stride) for j in range(k, len(base), stride)]

    def kv_copy(h, u):
        src = k_hbm if u < per_head // 2 else v_hbm
        s, r = divmod(u % (per_head // 2), nr)
        return pltpu.make_async_copy(
            src.at[h, pl.ds(r * ROWS, ROWS), pl.ds(w0 + s * SCH, SCH)],
            kv.at[u % NSLOT], sems.at[u % NSLOT])

    def weight_jobs(pairs, job, first):
        def make(src, dst, i):
            return lambda: pltpu.make_async_copy(src, dst, sems.at[i % NSLOT])
        return [(make(src, dst, first + i), job[0] * job[1] * 2) for i, (src, dst) in enumerate(pairs)]

    def kv_jobs(h, lo, hi):
        return [(functools.partial(kv_copy, h, u), kv_bytes) for u in range(lo, hi)]

    def concat(lists, first):
        out = []
        for pairs, job in lists:
            out += weight_jobs(pairs, job, first + len(out))
        return out

    wm_t, wq_t, wo_t = tiles(wm_hbm, wm_v, WM_JOB), tiles(wq_hbm, wq_v, WQ_JOB), tiles(wo_hbm, wo_v, WO_JOB)
    wg_t, wu_t, wd_t = tiles(wg_hbm, wg_v, WGU_JOB), tiles(wu_hbm, wu_v, WGU_JOB), tiles(wd_hbm, wd_v, WD_JOB)
    n_pre = len(wm_t) + len(wq_t) + len(wo_t)
    pre = concat([(wm_t, WM_JOB), (wq_t, WQ_JOB), (wo_t, WO_JOB)], -n_pre)
    post = concat([(wg_t, WGU_JOB), (wu_t, WGU_JOB), (wd_t, WD_JOB)], 0)
    assert budget // min(n for _, n in pre + post) <= NSLOT

    x_cp = pltpu.make_async_copy(x_hbm, x_v, small_sems.at[0])
    c_cp = pltpu.make_async_copy(c_hbm, c_v, small_sems.at[1])
    c_cp.start()
    x_cp.start()
    st = _Stream(pre + kv_jobs(0, 0, LOOKAHEAD), -n_pre, budget)
    st.fill()
    c_cp.wait()
    x_cp.wait()
    c = _bcast_rows(c_v[...].astype(F32))
    sc = (c * jax.nn.sigmoid(c)).astype(BF16)
    x = _bcast_rows(x_v[...].astype(F32))
    lnx = _layernorm(x)

    def mxu(a, w):
        return jnp.dot(a, w, preferred_element_type=F32)

    st.step(len(wm_t))
    cols = range(0, 6 * D, MOD_COLS)
    for c0 in cols:
        mod_s[:, c0:c0 + MOD_COLS] = mxu(sc, wm_v[:, c0:c0 + MOD_COLS])
        st.step(len(wq_t) // (len(cols) + 1))
    sa, ca = mod_s[:, 0:D], mod_s[:, D:2 * D]
    hq = (lnx * (1.0 + ca) + sa).astype(BF16)
    st.step(len(wm_t) + len(wq_t) - st.waited)

    eye = (lax.broadcasted_iota(jnp.int32, (128, 128), 0)
           == lax.broadcasted_iota(jnp.int32, (128, 128), 1)).astype(F32).astype(BF16)
    cols = range(0, H * DH, Q_COLS)
    for c0 in cols:
        q = mxu(hq, wq_v[:, c0:c0 + Q_COLS]).astype(BF16)
        rep = jnp.concatenate([jnp.broadcast_to(q[0:1, t:t + 128], (128, 128))
                               for t in range(0, Q_COLS, 128)], axis=0)
        col = lax.dot_general(eye, rep, (((1,), (1,)), ((), ())), preferred_element_type=F32)
        for t in range(0, Q_COLS, 128):
            qb[c0 + t:c0 + t + 128, :] = col[:, t:t + 128] * np.float32(DH ** -0.5)
        st.step(len(wo_t) // (len(cols) + 1))
    st.step(n_pre - st.waited)
    assert st.started == n_pre + LOOKAHEAD

    def head(h, out_acc, last):
        if last:
            st = _Stream(kv_jobs(h, 0, per_head) + post, 0, budget, started=LOOKAHEAD)

        def kv_step(u):
            if last:
                st.step()
            else:
                kv_copy(h, u).wait()
                j = u + LOOKAHEAD
                nxt = kv_copy(h, j) if j < per_head else kv_copy(h + 1, j - per_head)
                nxt.start(priority=PRIO[j % len(PRIO)])
            return kv[u % NSLOT].astype(F32)

        row0 = h * DH
        sub = ROWS // 8

        def rows8(ref, r8):
            return ref[pl.ds(pl.multiple_of(row0 + r8 * 8, 8), 8), :]

        u = 0
        for s in range(ns):
            acc = jnp.zeros((8, SCH), F32)
            for r in range(nr):
                kt = kv_step(u)
                u += 1
                for i in range(sub):
                    qv = rows8(qb, r * sub + i)
                    acc = acc + kt[i * 8:(i + 1) * 8, :] * jnp.tile(qv, (1, SCH // 128))
            p_s[:, s * SCH:(s + 1) * SCH] = _bcast_rows(jnp.sum(acc, axis=0, keepdims=True))
        sc_all = p_s[...]
        m = jnp.max(sc_all, axis=-1, keepdims=True)
        p = jnp.exp(sc_all - m)
        l = jnp.sum(p, axis=-1, keepdims=True)
        p_s[...] = p
        oacc = [None] * (DH // 8)
        for s in range(ns):
            ps = p_s[:, s * SCH:(s + 1) * SCH]
            for r in range(nr):
                vt = kv_step(u)
                u += 1
                for i in range(sub):
                    prod = vt[i * 8:(i + 1) * 8, :] * ps
                    parts = [prod[:, t * 128:(t + 1) * 128] for t in range(SCH // 128)]
                    while len(parts) > 1:
                        parts = [parts[t] + parts[t + 1] for t in range(0, len(parts), 2)]
                    r8 = r * sub + i
                    oacc[r8] = parts[0] if s == 0 else oacc[r8] + parts[0]
        o = jnp.sum(jnp.concatenate(oacc, axis=0), axis=-1, keepdims=True) / l[0:1, :]
        ob = jnp.broadcast_to(o, (DH, 128))
        for r8 in range(DH // 8):
            wt = rows8(wo_v, r8).astype(F32)
            out_acc = out_acc + wt * jnp.tile(ob[r8 * 8:(r8 + 1) * 8, :], (1, D // 128))
        return (out_acc, st) if last else out_acc

    out_acc = lax.fori_loop(0, H - 1, lambda h, a: head(h, a, False), jnp.zeros((8, D), F32))
    out_acc, st = head(H - 1, out_acc, True)

    attn = _bcast_rows(jnp.sum(out_acc, axis=0, keepdims=True))
    ga, sb, cb, gb = (mod_s[:, i * D:(i + 1) * D] for i in (2, 3, 4, 5))
    x1 = x + ga * attn
    h2 = (_layernorm(x1) * (1.0 + cb) + sb).astype(BF16)
    st.step(len(wg_t))
    cols = range(0, F, FFN_COLS)
    gelu = []
    for c0 in cols:
        gelu.append(jax.nn.gelu(mxu(h2, wg_v[:, c0:c0 + FFN_COLS]), approximate=True))
        st.step(len(wu_t) // (len(cols) + 1))
    st.step(per_head + len(wg_t) + len(wu_t) - st.waited)
    first_wd = st.waited
    act = []
    for i, c0 in enumerate(cols):
        act.append((gelu[i] * mxu(h2, wu_v[:, c0:c0 + FFN_COLS])).astype(BF16))
        st.step(WD_SPLITS[0] // WD_JOB[0] // (len(cols) + 1))
    act = jnp.concatenate(act, axis=1)
    y, r0 = None, 0
    for r1 in WD_SPLITS:
        st.step(first_wd + r1 // WD_JOB[0] - st.waited)
        part = mxu(act[:, r0:r1], wd_v[r0:r1, :])
        y, r0 = (part if y is None else y + part), r1
    assert st.waited == len(st.jobs)
    o_ref[...] = (x1 + gb * y)[0:1, :].astype(o_ref.dtype)


@jax.jit
def pallas_adaLN_cond__sliding_block_cached__geglu_ffn__decode_kernel(
    A_x: jax.Array,
    A_k_cache: jax.Array,
    A_v_cache: jax.Array,
    A_wq: jax.Array,
    A_wo: jax.Array,
    B_x: jax.Array,
    B_w_gate: jax.Array,
    B_w_up: jax.Array,
    B_w_down: jax.Array,
    c: jax.Array,
    w_mod: jax.Array,
):
    del B_x
    _, hkv, sk, dh = A_k_cache.shape
    assert A_x.shape == (1, 1, D) and (hkv, dh) == (H, DH)
    window = min(WINDOW_MAX, max(256, sk // 4))
    assert window % SCH == 0

    k_t = jnp.transpose(A_k_cache, (0, 1, 3, 2)).reshape(H, DH, sk)
    v_t = jnp.transpose(A_v_cache, (0, 1, 3, 2)).reshape(H, DH, sk)

    hbm = pl.BlockSpec(memory_space=pl.ANY)
    out = pl.pallas_call(
        functools.partial(_kernel, sk=sk, window=window),
        out_shape=jax.ShapeDtypeStruct((1, D), A_x.dtype),
        in_specs=[hbm] * 10,
        out_specs=pl.BlockSpec(memory_space=pltpu.VMEM),
        scratch_shapes=[
            pltpu.VMEM((1, D), BF16),
            pltpu.VMEM((1, D), BF16),
            pltpu.VMEM((D, 6 * D), BF16),
            pltpu.VMEM((D, H * DH), BF16),
            pltpu.VMEM((H * DH, D), BF16),
            pltpu.VMEM((D, F), BF16),
            pltpu.VMEM((D, F), BF16),
            pltpu.VMEM((F, D), BF16),
            pltpu.VMEM((NSLOT, ROWS, SCH), BF16),
            pltpu.VMEM((H * DH, 128), F32),
            pltpu.VMEM((8, window), F32),
            pltpu.VMEM((8, 6 * D), F32),
            pltpu.SemaphoreType.DMA((NSLOT,)),
            pltpu.SemaphoreType.DMA((2,)),
        ],
        compiler_params=pltpu.CompilerParams(vmem_limit_bytes=64 * 1024 * 1024,
                                             disable_semaphore_checks=True),
        name="adaln_attn_geglu_decode",
    )(A_x.reshape(1, D), c, k_t, v_t, A_wq, A_wo, B_w_gate, B_w_up, B_w_down, w_mod)
    return out.reshape(1, 1, D)
```

```python
import functools

import jax
import jax.numpy as jnp
import numpy as np
from jax import lax
from jax.experimental import pallas as pl
from jax.experimental.pallas import tpu as pltpu

F32 = jnp.float32
BF16 = jnp.bfloat16

D = 640
H = 32
DH = 192
F = 1536
WINDOW_MAX = 4096

ROWS = 16
SCH = 512
LOOKAHEAD = 64
NSLOT = 96
W_BUDGET = 1024 * 1024
PRIO = (0, 1, 1)
WM_JOB = (8, 1280, 24)
WQ_JOB = (8, 2048, 16)
WO_JOB = (24, 640, 16)
WGU_JOB = (8, 1536, 10)
WD_JOB = (16, 640, 1)
MOD_COLS = 768
Q_COLS = 512
FFN_COLS = 512
WD_SPLITS = (512, 1024, 1408, 1536)


def _layernorm(x):
    m = jnp.mean(x, axis=-1, keepdims=True)
    xc = x - m
    v = jnp.mean(xc * xc, axis=-1, keepdims=True)
    return xc / jnp.sqrt(v + 1e-5)


def _bcast_rows(x):
    return jnp.broadcast_to(x, (8, x.shape[-1]))


class _Stream:
    def __init__(self, jobs, first, budget, started=0):
        self.jobs, self.first, self.budget = jobs, first, budget
        self.waited, self.started = 0, started

    def fill(self):
        inflight = sum(n for _, n in self.jobs[self.waited:self.started])
        while self.started < len(self.jobs):
            make, n = self.jobs[self.started]
            if inflight + n > self.budget:
                break
            make().start(priority=PRIO[(self.first + self.started) % len(PRIO)])
            inflight += n
            self.started += 1

    def step(self, n=1):
        for _ in range(n):
            self.jobs[self.waited][0]().wait()
            self.waited += 1
            self.fill()


def _kernel(x_hbm, c_hbm, k_hbm, v_hbm, wq_hbm, wo_hbm, wg_hbm, wu_hbm, wd_hbm, wm_hbm,
            o_ref,
            x_v, c_v, wm_v, wq_v, wo_v, wg_v, wu_v, wd_v, kv, qb, p_s, mod_s, y_s,
            sems, small_sems, *, sk, window):
    nr = DH // ROWS
    ns = window // SCH
    per_head = 2 * nr * ns
    assert per_head % NSLOT == 0 and per_head % len(PRIO) == 0 and LOOKAHEAD <= NSLOT
    w0 = sk - window
    kv_bytes = ROWS * SCH * 2

    def tiles(hbm, vmem, job):
        (rows, cols, stride), (n, m) = job, hbm.shape
        base = [(pl.ds(r, rows), pl.ds(c0, cols)) for r in range(0, n, rows) for c0 in range(0, m, cols)]
        return [(hbm.at[base[j]], vmem.at[base[j]])
                for k in range(stride) for j in range(k, len(base), stride)]

    def kv_copy(h, u):
        src = k_hbm if u < per_head // 2 else v_hbm
        s, r = divmod(u % (per_head // 2), nr)
        return pltpu.make_async_copy(
            src.at[h, pl.ds(r * ROWS, ROWS), pl.ds(w0 + s * SCH, SCH)],
            kv.at[u % NSLOT], sems.at[u % NSLOT])

    def weight_jobs(pairs, job, first):
        def make(src, dst, i):
            return lambda: pltpu.make_async_copy(src, dst, sems.at[i % NSLOT])
        return [(make(src, dst, first + i), job[0] * job[1] * 2) for i, (src, dst) in enumerate(pairs)]

    def kv_jobs(h, lo, hi):
        return [(functools.partial(kv_copy, h, u), kv_bytes) for u in range(lo, hi)]

    def concat(lists, first):
        out = []
        for pairs, job in lists:
            out += weight_jobs(pairs, job, first + len(out))
        return out

    wm_t, wq_t, wo_t = tiles(wm_hbm, wm_v, WM_JOB), tiles(wq_hbm, wq_v, WQ_JOB), tiles(wo_hbm, wo_v, WO_JOB)
    wg_t, wu_t, wd_t = tiles(wg_hbm, wg_v, WGU_JOB), tiles(wu_hbm, wu_v, WGU_JOB), tiles(wd_hbm, wd_v, WD_JOB)
    n_pre = len(wm_t) + len(wq_t) + len(wo_t)
    pre = concat([(wm_t, WM_JOB), (wq_t, WQ_JOB), (wo_t, WO_JOB)], -n_pre)
    post = concat([(wg_t, WGU_JOB), (wu_t, WGU_JOB), (wd_t, WD_JOB)], 0)
    assert W_BUDGET // min(kv_bytes, *(n for _, n in pre + post)) <= NSLOT

    x_cp = pltpu.make_async_copy(x_hbm, x_v, small_sems.at[0])
    c_cp = pltpu.make_async_copy(c_hbm, c_v, small_sems.at[1])
    c_cp.start()
    x_cp.start()
    st = _Stream(pre + kv_jobs(0, 0, LOOKAHEAD), -n_pre, W_BUDGET)
    st.fill()
    c_cp.wait()
    x_cp.wait()
    c = _bcast_rows(c_v[...].astype(F32))
    sc = (c * jax.nn.sigmoid(c)).astype(BF16)
    x = _bcast_rows(x_v[...].astype(F32))
    lnx = _layernorm(x)

    def mxu(a, w):
        return jnp.dot(a, w, preferred_element_type=F32)

    st.step(len(wm_t))
    cols = range(0, 6 * D, MOD_COLS)
    for c0 in cols:
        mod_s[:, c0:c0 + MOD_COLS] = mxu(sc, wm_v[:, c0:c0 + MOD_COLS])
        st.step(len(wq_t) // (len(cols) + 1))
    sa, ca = mod_s[:, 0:D], mod_s[:, D:2 * D]
    hq = (lnx * (1.0 + ca) + sa).astype(BF16)
    st.step(len(wm_t) + len(wq_t) - st.waited)

    eye = (lax.broadcasted_iota(jnp.int32, (128, 128), 0)
           == lax.broadcasted_iota(jnp.int32, (128, 128), 1)).astype(F32).astype(BF16)
    cols = range(0, H * DH, Q_COLS)
    for c0 in cols:
        q = mxu(hq, wq_v[:, c0:c0 + Q_COLS]).astype(BF16)
        rep = jnp.concatenate([jnp.broadcast_to(q[0:1, t:t + 128], (128, 128))
                               for t in range(0, Q_COLS, 128)], axis=0)
        col = lax.dot_general(eye, rep, (((1,), (1,)), ((), ())), preferred_element_type=F32)
        for t in range(0, Q_COLS, 128):
            qb[c0 + t:c0 + t + 128, :] = col[:, t:t + 128] * np.float32(DH ** -0.5)
        st.step(len(wo_t) // (len(cols) + 1))
    st.step(n_pre - st.waited)
    st.budget = LOOKAHEAD * kv_bytes
    st.fill()
    assert st.started == n_pre + LOOKAHEAD

    def head(h, out_acc, last):
        if last:
            st = _Stream(kv_jobs(h, 0, per_head) + post, 0, LOOKAHEAD * kv_bytes, started=LOOKAHEAD)

        def kv_step(u):
            if last:
                if u == per_head - LOOKAHEAD:
                    st.budget = W_BUDGET
                st.step()
            else:
                kv_copy(h, u).wait()
                j = u + LOOKAHEAD
                nxt = kv_copy(h, j) if j < per_head else kv_copy(h + 1, j - per_head)
                nxt.start(priority=PRIO[j % len(PRIO)])
            return kv[u % NSLOT].astype(F32)

        row0 = h * DH
        sub = ROWS // 8

        def rows8(ref, r8):
            return ref[pl.ds(pl.multiple_of(row0 + r8 * 8, 8), 8), :]

        u = 0
        for s in range(ns):
            acc = jnp.zeros((8, SCH), F32)
            for r in range(nr):
                kt = kv_step(u)
                u += 1
                for i in range(sub):
                    qv = rows8(qb, r * sub + i)
                    acc = acc + kt[i * 8:(i + 1) * 8, :] * jnp.tile(qv, (1, SCH // 128))
            p_s[:, s * SCH:(s + 1) * SCH] = _bcast_rows(jnp.sum(acc, axis=0, keepdims=True))
        sc_all = p_s[...]
        m = jnp.max(sc_all, axis=-1, keepdims=True)
        p = jnp.exp(sc_all - m)
        l = jnp.sum(p, axis=-1, keepdims=True)
        p_s[...] = p
        oacc = [None] * (DH // 8)
        for s in range(ns):
            ps = p_s[:, s * SCH:(s + 1) * SCH]
            for r in range(nr):
                vt = kv_step(u)
                u += 1
                for i in range(sub):
                    prod = vt[i * 8:(i + 1) * 8, :] * ps
                    parts = [prod[:, t * 128:(t + 1) * 128] for t in range(SCH // 128)]
                    while len(parts) > 1:
                        parts = [parts[t] + parts[t + 1] for t in range(0, len(parts), 2)]
                    r8 = r * sub + i
                    oacc[r8] = parts[0] if s == 0 else oacc[r8] + parts[0]
        o = jnp.sum(jnp.concatenate(oacc, axis=0), axis=-1, keepdims=True) / l[0:1, :]
        ob = jnp.broadcast_to(o, (DH, 128))
        for r8 in range(DH // 8):
            wt = rows8(wo_v, r8).astype(F32)
            out_acc = out_acc + wt * jnp.tile(ob[r8 * 8:(r8 + 1) * 8, :], (1, D // 128))
        return (out_acc, st) if last else out_acc

    out_acc = lax.fori_loop(0, H - 1, lambda h, a: head(h, a, False), jnp.zeros((8, D), F32))
    out_acc, st = head(H - 1, out_acc, True)

    attn = _bcast_rows(jnp.sum(out_acc, axis=0, keepdims=True))
    ga, sb, cb, gb = (mod_s[:, i * D:(i + 1) * D] for i in (2, 3, 4, 5))
    x1 = x + ga * attn
    h2 = (_layernorm(x1) * (1.0 + cb) + sb).astype(BF16)
    st.step(len(wg_t))
    cols = range(0, F, FFN_COLS)
    gelu = []
    for c0 in cols:
        gelu.append(jax.nn.gelu(mxu(h2, wg_v[:, c0:c0 + FFN_COLS]), approximate=True))
        st.step(len(wu_t) // (len(cols) + 1))
    st.step(per_head + len(wg_t) + len(wu_t) - st.waited)
    first_wd = st.waited
    act = []
    for i, c0 in enumerate(cols):
        act.append((gelu[i] * mxu(h2, wu_v[:, c0:c0 + FFN_COLS])).astype(BF16))
        st.step(WD_SPLITS[0] // WD_JOB[0] // (len(cols) + 1))
    act = jnp.concatenate(act, axis=1)
    r0 = 0
    for r1 in WD_SPLITS:
        st.step(first_wd + r1 // WD_JOB[0] - st.waited)
        part = mxu(act[:, r0:r1], wd_v[r0:r1, :])
        if r1 == F:
            y = y_s[...] + part
        elif r0 == 0:
            y_s[...] = part
        else:
            y_s[...] += part
        r0 = r1
    assert st.waited == len(st.jobs)
    o_ref[...] = (x1 + gb * y)[0:1, :].astype(o_ref.dtype)


@jax.jit
def pallas_adaLN_cond__sliding_block_cached__geglu_ffn__decode_kernel(
    A_x: jax.Array,
    A_k_cache: jax.Array,
    A_v_cache: jax.Array,
    A_wq: jax.Array,
    A_wo: jax.Array,
    B_x: jax.Array,
    B_w_gate: jax.Array,
    B_w_up: jax.Array,
    B_w_down: jax.Array,
    c: jax.Array,
    w_mod: jax.Array,
):
    del B_x
    _, hkv, sk, dh = A_k_cache.shape
    assert A_x.shape == (1, 1, D) and (hkv, dh) == (H, DH)
    window = min(WINDOW_MAX, max(256, sk // 4))
    assert window % SCH == 0

    k_t = jnp.transpose(A_k_cache, (0, 1, 3, 2)).reshape(H, DH, sk)
    v_t = jnp.transpose(A_v_cache, (0, 1, 3, 2)).reshape(H, DH, sk)

    hbm = pl.BlockSpec(memory_space=pl.ANY)
    out = pl.pallas_call(
        functools.partial(_kernel, sk=sk, window=window),
        out_shape=jax.ShapeDtypeStruct((1, D), A_x.dtype),
        in_specs=[hbm] * 10,
        out_specs=pl.BlockSpec(memory_space=pltpu.VMEM),
        scratch_shapes=[
            pltpu.VMEM((1, D), BF16),
            pltpu.VMEM((1, D), BF16),
            pltpu.VMEM((D, 6 * D), BF16),
            pltpu.VMEM((D, H * DH), BF16),
            pltpu.VMEM((H * DH, D), BF16),
            pltpu.VMEM((D, F), BF16),
            pltpu.VMEM((D, F), BF16),
            pltpu.VMEM((F, D), BF16),
            pltpu.VMEM((NSLOT, ROWS, SCH), BF16),
            pltpu.VMEM((H * DH, 128), F32),
            pltpu.VMEM((8, window), F32),
            pltpu.VMEM((8, 6 * D), F32),
            pltpu.VMEM((8, D), F32),
            pltpu.SemaphoreType.DMA((NSLOT,)),
            pltpu.SemaphoreType.DMA((2,)),
        ],
        compiler_params=pltpu.CompilerParams(vmem_limit_bytes=64 * 1024 * 1024,
                                             disable_semaphore_checks=True),
        name="adaln_attn_geglu_decode",
    )(A_x.reshape(1, D), c, k_t, v_t, A_wq, A_wo, B_w_gate, B_w_up, B_w_down, w_mod)
    return out.reshape(1, 1, D)
```

```python
import functools

import jax
import jax.numpy as jnp
import numpy as np
from jax import lax
from jax.experimental import pallas as pl
from jax.experimental.pallas import tpu as pltpu

F32 = jnp.float32
BF16 = jnp.bfloat16

D = 640
H = 32
DH = 192
F = 1536
WINDOW_MAX = 4096

ROWS = 16
SCH = 512
LOOKAHEAD = 64
NSLOT = 96
W_BUDGET = 1024 * 1024
PRIO = (1, 1, 0)
WM_JOB = (8, 1280, 24)
WQ_JOB = (8, 2048, 16)
WO_JOB = (24, 640, 16)
WGU_JOB = (8, 1536, 10)
WD_JOB = (16, 640, 1)
MOD_COLS = 768
Q_COLS = 512
FFN_COLS = 512
WD_SPLITS = (640, 1152, 1408)


def _layernorm(x):
    m = jnp.mean(x, axis=-1, keepdims=True)
    xc = x - m
    v = jnp.mean(xc * xc, axis=-1, keepdims=True)
    return xc / jnp.sqrt(v + 1e-5)


def _bcast_rows(x):
    return jnp.broadcast_to(x, (8, x.shape[-1]))


class _Stream:
    def __init__(self, jobs, first, budget, started=0):
        self.jobs, self.first, self.budget = jobs, first, budget
        self.waited, self.started = 0, started

    def fill(self):
        inflight = sum(n for _, n in self.jobs[self.waited:self.started])
        while self.started < len(self.jobs):
            make, n = self.jobs[self.started]
            if inflight + n > self.budget:
                break
            make().start(priority=PRIO[(self.first + self.started) % len(PRIO)])
            inflight += n
            self.started += 1

    def step(self, n=1):
        for _ in range(n):
            self.jobs[self.waited][0]().wait()
            self.waited += 1
            self.fill()


def _kernel(x_hbm, c_hbm, k_hbm, v_hbm, wq_hbm, wo_hbm, wg_hbm, wu_hbm, wd_hbm, wm_hbm,
            o_ref,
            x_v, c_v, wm_v, wq_v, wo_v, wg_v, wu_v, wd_v, kv, qb, p_s, mod_s, y_s, acol_s,
            sems, small_sems, *, sk, window):
    nr = DH // ROWS
    ns = window // SCH
    per_head = 2 * nr * ns
    assert per_head % NSLOT == 0 and per_head % len(PRIO) == 0 and LOOKAHEAD <= NSLOT
    w0 = sk - window
    kv_bytes = ROWS * SCH * 2

    def tiles(hbm, vmem, job):
        (rows, cols, stride), (n, m) = job, hbm.shape
        base = [(pl.ds(r, rows), pl.ds(c0, cols)) for r in range(0, n, rows) for c0 in range(0, m, cols)]
        return [(hbm.at[base[j]], vmem.at[base[j]])
                for k in range(stride) for j in range(k, len(base), stride)]

    def kv_copy(h, u):
        src = k_hbm if u < per_head // 2 else v_hbm
        s, r = divmod(u % (per_head // 2), nr)
        return pltpu.make_async_copy(
            src.at[h, pl.ds(r * ROWS, ROWS), pl.ds(w0 + s * SCH, SCH)],
            kv.at[u % NSLOT], sems.at[u % NSLOT])

    def weight_jobs(pairs, job, first):
        def make(src, dst, i):
            return lambda: pltpu.make_async_copy(src, dst, sems.at[i % NSLOT])
        return [(make(src, dst, first + i), job[0] * job[1] * 2) for i, (src, dst) in enumerate(pairs)]

    def kv_jobs(h, lo, hi):
        return [(functools.partial(kv_copy, h, u), kv_bytes) for u in range(lo, hi)]

    def concat(lists, first):
        out = []
        for pairs, job in lists:
            out += weight_jobs(pairs, job, first + len(out))
        return out

    wm_t, wq_t, wo_t = tiles(wm_hbm, wm_v, WM_JOB), tiles(wq_hbm, wq_v, WQ_JOB), tiles(wo_hbm, wo_v, WO_JOB)
    wg_t, wu_t, wd_t = tiles(wg_hbm, wg_v, WGU_JOB), tiles(wu_hbm, wu_v, WGU_JOB), tiles(wd_hbm, wd_v, WD_JOB)
    n_pre = len(wm_t) + len(wq_t) + len(wo_t) + len(wg_t)
    pre = concat([(wm_t, WM_JOB), (wq_t, WQ_JOB), (wo_t, WO_JOB), (wg_t, WGU_JOB)], -n_pre)
    post = concat([(wu_t, WGU_JOB), (wd_t, WD_JOB)], 0)
    assert W_BUDGET // min(kv_bytes, *(n for _, n in pre + post)) <= NSLOT

    x_cp = pltpu.make_async_copy(x_hbm, x_v, small_sems.at[0])
    c_cp = pltpu.make_async_copy(c_hbm, c_v, small_sems.at[1])
    c_cp.start()
    x_cp.start()
    st = _Stream(pre + kv_jobs(0, 0, LOOKAHEAD), -n_pre, W_BUDGET)
    st.fill()
    c_cp.wait()
    x_cp.wait()
    c = _bcast_rows(c_v[...].astype(F32))
    sc = (c * jax.nn.sigmoid(c)).astype(BF16)
    x = _bcast_rows(x_v[...].astype(F32))
    lnx = _layernorm(x)

    def mxu(a, w):
        return jnp.dot(a, w, preferred_element_type=F32)

    st.step(len(wm_t))
    cols = range(0, 6 * D, MOD_COLS)
    for c0 in cols:
        mod_s[:, c0:c0 + MOD_COLS] = mxu(sc, wm_v[:, c0:c0 + MOD_COLS])
        st.step(len(wq_t) // (len(cols) + 1))
    sa, ca = mod_s[:, 0:D], mod_s[:, D:2 * D]
    hq = (lnx * (1.0 + ca) + sa).astype(BF16)
    st.step(len(wm_t) + len(wq_t) - st.waited)

    eye = (lax.broadcasted_iota(jnp.int32, (128, 128), 0)
           == lax.broadcasted_iota(jnp.int32, (128, 128), 1)).astype(F32).astype(BF16)

    def columns(row):
        n = row.shape[1]
        rep = jnp.concatenate([jnp.broadcast_to(row[0:1, t:t + 128], (128, 128))
                               for t in range(0, n, 128)], axis=0)
        col = lax.dot_general(eye, rep, (((1,), (1,)), ((), ())), preferred_element_type=F32)
        return [col[:, t:t + 128] for t in range(0, n, 128)]

    cols = range(0, H * DH, Q_COLS)
    n_each = (n_pre - st.waited) // (len(cols) + 1)
    for c0 in cols:
        q = mxu(hq, wq_v[:, c0:c0 + Q_COLS])
        st.step(n_each // 3)
        blocks = columns(q.astype(BF16))
        st.step(n_each // 3)
        for i, blk in enumerate(blocks):
            qb[c0 + i * 128:c0 + (i + 1) * 128, :] = blk * np.float32(DH ** -0.5)
        st.step(n_each - 2 * (n_each // 3))
    st.step(n_pre - st.waited)
    st.budget = LOOKAHEAD * kv_bytes
    st.fill()
    assert st.started == n_pre + LOOKAHEAD

    def head(h, out_acc, last):
        if last:
            st = _Stream(kv_jobs(h, 0, per_head) + post, 0, LOOKAHEAD * kv_bytes, started=LOOKAHEAD)

        def kv_step(u):
            if last:
                if u == per_head - LOOKAHEAD:
                    st.budget = W_BUDGET
                st.step()
            else:
                kv_copy(h, u).wait()
                j = u + LOOKAHEAD
                nxt = kv_copy(h, j) if j < per_head else kv_copy(h + 1, j - per_head)
                nxt.start(priority=PRIO[j % len(PRIO)])
            return kv[u % NSLOT].astype(F32)

        row0 = h * DH
        sub = ROWS // 8

        def rows8(ref, r8):
            return ref[pl.ds(pl.multiple_of(row0 + r8 * 8, 8), 8), :]

        u = 0
        for s in range(ns):
            acc = jnp.zeros((8, SCH), F32)
            for r in range(nr):
                kt = kv_step(u)
                u += 1
                for i in range(sub):
                    qv = rows8(qb, r * sub + i)
                    acc = acc + kt[i * 8:(i + 1) * 8, :] * jnp.tile(qv, (1, SCH // 128))
            p_s[:, s * SCH:(s + 1) * SCH] = _bcast_rows(jnp.sum(acc, axis=0, keepdims=True))
        sc_all = p_s[...]
        m = jnp.max(sc_all, axis=-1, keepdims=True)
        p = jnp.exp(sc_all - m)
        l = jnp.sum(p, axis=-1, keepdims=True)
        p_s[...] = p
        oacc = [None] * (DH // 8)
        for s in range(ns):
            ps = p_s[:, s * SCH:(s + 1) * SCH]
            for r in range(nr):
                vt = kv_step(u)
                u += 1
                for i in range(sub):
                    prod = vt[i * 8:(i + 1) * 8, :] * ps
                    parts = [prod[:, t * 128:(t + 1) * 128] for t in range(SCH // 128)]
                    while len(parts) > 1:
                        parts = [parts[t] + parts[t + 1] for t in range(0, len(parts), 2)]
                    r8 = r * sub + i
                    oacc[r8] = parts[0] if s == 0 else oacc[r8] + parts[0]
        o = jnp.sum(jnp.concatenate(oacc, axis=0), axis=-1, keepdims=True) / l[0:1, :]
        ob = jnp.broadcast_to(o, (DH, 128))
        for r8 in range(DH // 8):
            wt = rows8(wo_v, r8).astype(F32)
            out_acc = out_acc + wt * jnp.tile(ob[r8 * 8:(r8 + 1) * 8, :], (1, D // 128))
        return (out_acc, st) if last else out_acc

    out_acc = lax.fori_loop(0, H - 1, lambda h, a: head(h, a, False), jnp.zeros((8, D), F32))
    out_acc, st = head(H - 1, out_acc, True)

    attn = _bcast_rows(jnp.sum(out_acc, axis=0, keepdims=True))
    ga, sb, cb, gb = (mod_s[:, i * D:(i + 1) * D] for i in (2, 3, 4, 5))
    x1 = x + ga * attn
    h2 = (_layernorm(x1) * (1.0 + cb) + sb).astype(BF16)
    cols = range(0, F, FFN_COLS)
    gelu = []
    for c0 in cols:
        gelu.append(jax.nn.gelu(mxu(h2, wg_v[:, c0:c0 + FFN_COLS]), approximate=True))
        st.step(len(wu_t) // (len(cols) + 1))
    first_wd = per_head + len(wu_t)
    st.step(first_wd - st.waited)
    act = []
    for i, c0 in enumerate(cols):
        act.append((gelu[i] * mxu(h2, wu_v[:, c0:c0 + FFN_COLS])).astype(BF16))
        st.step(WD_SPLITS[0] // WD_JOB[0] // (len(cols) + 1))
    act = jnp.concatenate(act, axis=1)
    acol_s[...] = columns(act[:, F - 128:])[0]
    r0 = 0
    for r1 in WD_SPLITS:
        st.step(first_wd + r1 // WD_JOB[0] - st.waited)
        part = mxu(act[:, r0:r1], wd_v[r0:r1, :])
        if r0 == 0:
            y_s[...] = part
        else:
            y_s[...] += part
        r0 = r1
    assert r0 == F - 128
    y = jnp.zeros((8, D), F32)
    for r in range(r0, F, 8):
        if r % WD_JOB[0] == 0:
            st.step()
        y = y + wd_v[r:r + 8, :].astype(F32) * jnp.tile(acol_s[r - r0:r - r0 + 8, :], (1, D // 128))
    y = y_s[...] + _bcast_rows(jnp.sum(y, axis=0, keepdims=True))
    assert st.waited == len(st.jobs)
    o_ref[...] = (x1 + gb * y)[0:1, :].astype(o_ref.dtype)


@jax.jit
def pallas_adaLN_cond__sliding_block_cached__geglu_ffn__decode_kernel(
    A_x: jax.Array,
    A_k_cache: jax.Array,
    A_v_cache: jax.Array,
    A_wq: jax.Array,
    A_wo: jax.Array,
    B_x: jax.Array,
    B_w_gate: jax.Array,
    B_w_up: jax.Array,
    B_w_down: jax.Array,
    c: jax.Array,
    w_mod: jax.Array,
):
    del B_x
    _, hkv, sk, dh = A_k_cache.shape
    assert A_x.shape == (1, 1, D) and (hkv, dh) == (H, DH)
    window = min(WINDOW_MAX, max(256, sk // 4))
    assert window % SCH == 0

    k_t = jnp.transpose(A_k_cache, (0, 1, 3, 2)).reshape(H, DH, sk)
    v_t = jnp.transpose(A_v_cache, (0, 1, 3, 2)).reshape(H, DH, sk)

    hbm = pl.BlockSpec(memory_space=pl.ANY)
    out = pl.pallas_call(
        functools.partial(_kernel, sk=sk, window=window),
        out_shape=jax.ShapeDtypeStruct((1, D), A_x.dtype),
        in_specs=[hbm] * 10,
        out_specs=pl.BlockSpec(memory_space=pltpu.VMEM),
        scratch_shapes=[
            pltpu.VMEM((1, D), BF16),
            pltpu.VMEM((1, D), BF16),
            pltpu.VMEM((D, 6 * D), BF16),
            pltpu.VMEM((D, H * DH), BF16),
            pltpu.VMEM((H * DH, D), BF16),
            pltpu.VMEM((D, F), BF16),
            pltpu.VMEM((D, F), BF16),
            pltpu.VMEM((F, D), BF16),
            pltpu.VMEM((NSLOT, ROWS, SCH), BF16),
            pltpu.VMEM((H * DH, 128), F32),
            pltpu.VMEM((8, window), F32),
            pltpu.VMEM((8, 6 * D), F32),
            pltpu.VMEM((8, D), F32),
            pltpu.VMEM((128, 128), F32),
            pltpu.SemaphoreType.DMA((NSLOT,)),
            pltpu.SemaphoreType.DMA((2,)),
        ],
        compiler_params=pltpu.CompilerParams(vmem_limit_bytes=64 * 1024 * 1024,
                                             disable_semaphore_checks=True),
        name="adaln_attn_geglu_decode",
    )(A_x.reshape(1, D), c, k_t, v_t, A_wq, A_wo, B_w_gate, B_w_up, B_w_down, w_mod)
    return out.reshape(1, 1, D)
```

```python
import functools

import jax
import jax.numpy as jnp
import numpy as np
from jax import lax
from jax.experimental import pallas as pl
from jax.experimental.pallas import tpu as pltpu

F32 = jnp.float32
BF16 = jnp.bfloat16

D = 640
H = 32
DH = 192
F = 1536
WINDOW_MAX = 4096

ROWS = 16
SCH = 512
LOOKAHEAD = 64
NSLOT = 96
W_BUDGET = 1024 * 1024
PRIO = (1, 1, 0)
WM_JOB = (8, 1280, 24)
WQ_JOB = (8, 2048, 16)
WO_JOB = (24, 640, 16)
WGU_JOB = (8, 1536, 10)
WD_JOB = (16, 640, 1)
MOD_COLS = 768
Q_COLS = 512
FFN_COLS = 512
GAP_STEPS = 6
WD_STEPS = 8


def _layernorm(x):
    m = jnp.mean(x, axis=-1, keepdims=True)
    xc = x - m
    v = jnp.mean(xc * xc, axis=-1, keepdims=True)
    return xc / jnp.sqrt(v + 1e-5)


def _bcast_rows(x):
    return jnp.broadcast_to(x, (8, x.shape[-1]))


class _Stream:
    def __init__(self, jobs, first, budget, started=0):
        self.jobs, self.first, self.budget = jobs, first, budget
        self.waited, self.started = 0, started

    def fill(self):
        inflight = sum(n for _, n in self.jobs[self.waited:self.started])
        while self.started < len(self.jobs):
            make, n = self.jobs[self.started]
            if inflight + n > self.budget:
                break
            make().start(priority=PRIO[(self.first + self.started) % len(PRIO)])
            inflight += n
            self.started += 1

    def step(self, n=1):
        for _ in range(n):
            self.jobs[self.waited][0]().wait()
            self.waited += 1
            self.fill()


def _kernel(x_hbm, c_hbm, k_hbm, v_hbm, wq_hbm, wo_hbm, wg_hbm, wu_hbm, wd_hbm, wm_hbm,
            o_ref,
            x_v, c_v, wm_v, wq_v, wo_v, wg_v, wu_v, wd_v, kv, qb, p_s, mod_s, acol_s,
            sems, small_sems, *, sk, window):
    nr = DH // ROWS
    ns = window // SCH
    per_head = 2 * nr * ns
    assert per_head % NSLOT == 0 and per_head % len(PRIO) == 0 and LOOKAHEAD <= NSLOT
    w0 = sk - window
    kv_bytes = ROWS * SCH * 2

    def tiles(hbm, vmem, job):
        (rows, cols, stride), (n, m) = job, hbm.shape
        base = [(pl.ds(r, rows), pl.ds(c0, cols)) for r in range(0, n, rows) for c0 in range(0, m, cols)]
        order = [base[j] for k in range(stride) for j in range(k, len(base), stride)]
        return [(hbm.at[t], vmem.at[t]) for t in order], [t[0].start for t in order]

    def kv_copy(h, u):
        src = k_hbm if u < per_head // 2 else v_hbm
        s, r = divmod(u % (per_head // 2), nr)
        return pltpu.make_async_copy(
            src.at[h, pl.ds(r * ROWS, ROWS), pl.ds(w0 + s * SCH, SCH)],
            kv.at[u % NSLOT], sems.at[u % NSLOT])

    def weight_jobs(pairs, job, first):
        def make(src, dst, i):
            return lambda: pltpu.make_async_copy(src, dst, sems.at[i % NSLOT])
        return [(make(src, dst, first + i), job[0] * job[1] * 2) for i, (src, dst) in enumerate(pairs)]

    def kv_jobs(h, lo, hi):
        return [(functools.partial(kv_copy, h, u), kv_bytes) for u in range(lo, hi)]

    def concat(lists, first):
        out = []
        for pairs, job in lists:
            out += weight_jobs(pairs, job, first + len(out))
        return out

    (wm_t, _), (wq_t, _), (wo_t, _) = tiles(wm_hbm, wm_v, WM_JOB), tiles(wq_hbm, wq_v, WQ_JOB), tiles(wo_hbm, wo_v, WO_JOB)
    (wg_t, _), (wu_t, wu_rows), (wd_t, _) = tiles(wg_hbm, wg_v, WGU_JOB), tiles(wu_hbm, wu_v, WGU_JOB), tiles(wd_hbm, wd_v, WD_JOB)
    assert WGU_JOB[1] == F and WD_JOB[1:] == (D, 1)
    n_pre = len(wm_t) + len(wq_t) + len(wo_t) + len(wg_t)
    pre = concat([(wm_t, WM_JOB), (wq_t, WQ_JOB), (wo_t, WO_JOB), (wg_t, WGU_JOB)], -n_pre)
    post = concat([(wu_t, WGU_JOB), (wd_t, WD_JOB)], 0)
    assert W_BUDGET // min(kv_bytes, *(n for _, n in pre + post)) <= NSLOT

    x_cp = pltpu.make_async_copy(x_hbm, x_v, small_sems.at[0])
    c_cp = pltpu.make_async_copy(c_hbm, c_v, small_sems.at[1])
    c_cp.start()
    x_cp.start()
    st = _Stream(pre + kv_jobs(0, 0, LOOKAHEAD), -n_pre, W_BUDGET)
    st.fill()
    c_cp.wait()
    x_cp.wait()
    c = _bcast_rows(c_v[...].astype(F32))
    sc = (c * jax.nn.sigmoid(c)).astype(BF16)
    x = _bcast_rows(x_v[...].astype(F32))
    lnx = _layernorm(x)

    def mxu(a, w):
        return jnp.dot(a, w, preferred_element_type=F32)

    st.step(len(wm_t))
    cols = range(0, 6 * D, MOD_COLS)
    for c0 in cols:
        mod_s[:, c0:c0 + MOD_COLS] = mxu(sc, wm_v[:, c0:c0 + MOD_COLS])
        st.step(len(wq_t) // (len(cols) + 1))
    sa, ca = mod_s[:, 0:D], mod_s[:, D:2 * D]
    hq = (lnx * (1.0 + ca) + sa).astype(BF16)
    st.step(len(wm_t) + len(wq_t) - st.waited)

    eye = (lax.broadcasted_iota(jnp.int32, (128, 128), 0)
           == lax.broadcasted_iota(jnp.int32, (128, 128), 1)).astype(F32).astype(BF16)

    def columns(row):
        n = row.shape[1]
        rep = jnp.concatenate([jnp.broadcast_to(row[0:1, t:t + 128], (128, 128))
                               for t in range(0, n, 128)], axis=0)
        col = lax.dot_general(eye, rep, (((1,), (1,)), ((), ())), preferred_element_type=F32)
        return [col[:, t:t + 128] for t in range(0, n, 128)]

    cols = range(0, H * DH, Q_COLS)
    n_each = (n_pre - st.waited) // (len(cols) + 1)
    for c0 in cols:
        q = mxu(hq, wq_v[:, c0:c0 + Q_COLS])
        st.step(n_each // 3)
        blocks = columns(q.astype(BF16))
        st.step(n_each // 3)
        for i, blk in enumerate(blocks):
            qb[c0 + i * 128:c0 + (i + 1) * 128, :] = blk * np.float32(DH ** -0.5)
        st.step(n_each - 2 * (n_each // 3))
    st.step(n_pre - st.waited)
    st.budget = LOOKAHEAD * kv_bytes
    st.fill()
    assert st.started == n_pre + LOOKAHEAD

    def head(h, out_acc, last):
        if last:
            st = _Stream(kv_jobs(h, 0, per_head) + post, 0, LOOKAHEAD * kv_bytes, started=LOOKAHEAD)

        def kv_step(u):
            if last:
                if u == per_head - LOOKAHEAD:
                    st.budget = W_BUDGET
                st.step()
            else:
                kv_copy(h, u).wait()
                j = u + LOOKAHEAD
                nxt = kv_copy(h, j) if j < per_head else kv_copy(h + 1, j - per_head)
                nxt.start(priority=PRIO[j % len(PRIO)])
            return kv[u % NSLOT].astype(F32)

        row0 = h * DH
        sub = ROWS // 8

        def rows8(ref, r8):
            return ref[pl.ds(pl.multiple_of(row0 + r8 * 8, 8), 8), :]

        u = 0
        for s in range(ns):
            acc = jnp.zeros((8, SCH), F32)
            for r in range(nr):
                kt = kv_step(u)
                u += 1
                for i in range(sub):
                    qv = rows8(qb, r * sub + i)
                    acc = acc + kt[i * 8:(i + 1) * 8, :] * jnp.tile(qv, (1, SCH // 128))
            p_s[:, s * SCH:(s + 1) * SCH] = _bcast_rows(jnp.sum(acc, axis=0, keepdims=True))
        sc_all = p_s[...]
        m = jnp.max(sc_all, axis=-1, keepdims=True)
        p = jnp.exp(sc_all - m)
        l = jnp.sum(p, axis=-1, keepdims=True)
        p_s[...] = p
        oacc = [None] * (DH // 8)
        for s in range(ns):
            ps = p_s[:, s * SCH:(s + 1) * SCH]
            for r in range(nr):
                vt = kv_step(u)
                u += 1
                for i in range(sub):
                    prod = vt[i * 8:(i + 1) * 8, :] * ps
                    parts = [prod[:, t * 128:(t + 1) * 128] for t in range(SCH // 128)]
                    while len(parts) > 1:
                        parts = [parts[t] + parts[t + 1] for t in range(0, len(parts), 2)]
                    r8 = r * sub + i
                    oacc[r8] = parts[0] if s == 0 else oacc[r8] + parts[0]
        o = jnp.sum(jnp.concatenate(oacc, axis=0), axis=-1, keepdims=True) / l[0:1, :]
        ob = jnp.broadcast_to(o, (DH, 128))
        if last:
            st.step(GAP_STEPS)
        for r8 in range(DH // 8):
            wt = rows8(wo_v, r8).astype(F32)
            out_acc = out_acc + wt * jnp.tile(ob[r8 * 8:(r8 + 1) * 8, :], (1, D // 128))
        return (out_acc, st) if last else out_acc

    out_acc = lax.fori_loop(0, H - 1, lambda h, a: head(h, a, False), jnp.zeros((8, D), F32))
    out_acc, st = head(H - 1, out_acc, True)

    st.step(GAP_STEPS)
    attn = _bcast_rows(jnp.sum(out_acc, axis=0, keepdims=True))
    ga, sb, cb, gb = (mod_s[:, i * D:(i + 1) * D] for i in (2, 3, 4, 5))
    x1 = x + ga * attn
    h2 = (_layernorm(x1) * (1.0 + cb) + sb).astype(BF16)

    def row_tile(ref, r):
        w = ref[r:r + 8, :].astype(F32)
        return w * jnp.tile(acol_s[r:r + 8, :], (1, w.shape[1] // 128))

    st.step(GAP_STEPS)
    for i, blk in enumerate(columns(h2)):
        acol_s[i * 128:(i + 1) * 128, :] = blk
    g = jnp.zeros((8, F), F32)
    up = jnp.zeros((8, F), F32)
    done = 0
    while done < len(wu_rows):
        if st.waited < per_head + len(wu_rows):
            st.step()
        for _ in range(2):
            if done < min(len(wu_rows), st.waited - per_head):
                for r in range(wu_rows[done], wu_rows[done] + WGU_JOB[0], 8):
                    up = up + row_tile(wu_v, r)
                    g = g + row_tile(wg_v, r)
                done += 1
    st.step(GAP_STEPS)
    g = _bcast_rows(jnp.sum(g, axis=0, keepdims=True))
    up = _bcast_rows(jnp.sum(up, axis=0, keepdims=True))
    act = (jax.nn.gelu(g, approximate=True) * up).astype(BF16)
    st.step(GAP_STEPS)
    first_wd = per_head + len(wu_rows)
    n_wd = F // WD_JOB[0]
    y = jnp.zeros((8, D), F32)
    done = 0
    for c0 in range(0, F, FFN_COLS):
        for i, blk in enumerate(columns(act[:, c0:c0 + FFN_COLS])):
            acol_s[c0 + i * 128:c0 + (i + 1) * 128, :] = blk
        last_piece = c0 + FFN_COLS >= F
        avail = (c0 + FFN_COLS) // WD_JOB[0]
        for _ in range(n_wd - (st.waited - first_wd) if last_piece else WD_STEPS):
            st.step()
            for _ in range(3):
                if done < min(avail, st.waited - first_wd):
                    for r in range(done * WD_JOB[0], (done + 1) * WD_JOB[0], 8):
                        y = y + row_tile(wd_v, r)
                    done += 1
    assert done == n_wd
    y = _bcast_rows(jnp.sum(y, axis=0, keepdims=True))
    assert st.waited == len(st.jobs)
    o_ref[...] = (x1 + gb * y)[0:1, :].astype(o_ref.dtype)


@jax.jit
def pallas_adaLN_cond__sliding_block_cached__geglu_ffn__decode_kernel(
    A_x: jax.Array,
    A_k_cache: jax.Array,
    A_v_cache: jax.Array,
    A_wq: jax.Array,
    A_wo: jax.Array,
    B_x: jax.Array,
    B_w_gate: jax.Array,
    B_w_up: jax.Array,
    B_w_down: jax.Array,
    c: jax.Array,
    w_mod: jax.Array,
):
    del B_x
    _, hkv, sk, dh = A_k_cache.shape
    assert A_x.shape == (1, 1, D) and (hkv, dh) == (H, DH)
    window = min(WINDOW_MAX, max(256, sk // 4))
    assert window % SCH == 0

    k_t = jnp.transpose(A_k_cache, (0, 1, 3, 2)).reshape(H, DH, sk)
    v_t = jnp.transpose(A_v_cache, (0, 1, 3, 2)).reshape(H, DH, sk)

    hbm = pl.BlockSpec(memory_space=pl.ANY)
    out = pl.pallas_call(
        functools.partial(_kernel, sk=sk, window=window),
        out_shape=jax.ShapeDtypeStruct((1, D), A_x.dtype),
        in_specs=[hbm] * 10,
        out_specs=pl.BlockSpec(memory_space=pltpu.VMEM),
        scratch_shapes=[
            pltpu.VMEM((1, D), BF16),
            pltpu.VMEM((1, D), BF16),
            pltpu.VMEM((D, 6 * D), BF16),
            pltpu.VMEM((D, H * DH), BF16),
            pltpu.VMEM((H * DH, D), BF16),
            pltpu.VMEM((D, F), BF16),
            pltpu.VMEM((D, F), BF16),
            pltpu.VMEM((F, D), BF16),
            pltpu.VMEM((NSLOT, ROWS, SCH), BF16),
            pltpu.VMEM((H * DH, 128), F32),
            pltpu.VMEM((8, window), F32),
            pltpu.VMEM((8, 6 * D), F32),
            pltpu.VMEM((F, 128), F32),
            pltpu.SemaphoreType.DMA((NSLOT,)),
            pltpu.SemaphoreType.DMA((2,)),
        ],
        compiler_params=pltpu.CompilerParams(vmem_limit_bytes=64 * 1024 * 1024,
                                             disable_semaphore_checks=True),
        name="adaln_attn_geglu_decode",
    )(A_x.reshape(1, D), c, k_t, v_t, A_wq, A_wo, B_w_gate, B_w_up, B_w_down, w_mod)
    return out.reshape(1, 1, D)
```
